```python
import os as _os
_os.environ.setdefault("JAX_PLATFORMS", "cpu")
import jax
import jax.numpy as jnp

def _softmax(x, axis=-1):
    return jax.nn.softmax(x, axis=axis)
def _gelu(x):
    return jax.nn.gelu(x, approximate=True)
def _silu(x):
    return jax.nn.silu(x)
def _sigmoid(x):
    return jax.nn.sigmoid(x)
def _layernorm(x, axis=-1, eps=1e-5):
    m = jnp.mean(x, axis=axis, keepdims=True)
    v = jnp.var(x, axis=axis, keepdims=True)
    return (x - m) / jnp.sqrt(v + eps)
def _scatter_add(tgt, idx, src, axis=0):
    return tgt.at[idx].add(src)
def _segment_sum(src, seg, n):
    return jax.ops.segment_sum(src, seg, n)
class _Rng:
    def __init__(self, key):
        self._k = key
    def _next(self):
        self._k, sub = jax.random.split(self._k)
        return sub
    def normal(self, shape):
        return jax.random.normal(self._next(), shape, dtype=jnp.bfloat16)
    def randint(self, lo, hi, shape):
        return jax.random.randint(self._next(), shape, lo, hi, dtype=jnp.int32)
    def uniform(self, shape, lo=0.0, hi=1.0):
        return jax.random.uniform(self._next(), shape, jnp.bfloat16, lo, hi)
    def permutation(self, n):
        return jax.random.permutation(self._next(), n)


kernel_name = 'concat_heads__sliding_local_dilated__sliding_block__prompt'

def setup_inputs():
    _rng = _Rng(jax.random.key(int.from_bytes(__import__("os").urandom(4), "little")))
    _w = (lambda a: (lambda t: t.astype(jnp.bfloat16) if jnp.issubdtype(t.dtype, jnp.floating) else t)(jnp.asarray(a)))
    def _A_setup():
        B, S, D = 1, 2048, 1024
        return {
            "x": _w((lambda *s: _rng.normal(s) * 0.2)(B, S, D)),
            "wqkv": _w((lambda *s: _rng.normal(s) * 0.2)(D, 3 * D)),
            "wo": _w((lambda *s: _rng.normal(s) * 0.05)(D, D)),
        }
    _A_in = _A_setup()

    def _B_setup():
        B, S, D = 1, 2048, 1024
        return {
            "x": _w((lambda *s: _rng.normal(s) * 0.2)(B, S, D)),
            "wqkv": _w((lambda *s: _rng.normal(s) * 0.2)(D, 3 * D)),
            "wo": _w((lambda *s: _rng.normal(s) * 0.05)(D, D)),
        }
    _B_in = _B_setup()

    return {
        "A_x": _A_in["x"],
        "A_wqkv": _A_in["wqkv"],
        "A_wo": _A_in["wo"],
        "B_x": _B_in["x"],
        "B_wqkv": _B_in["wqkv"],
        "B_wo": _B_in["wo"],
    }

def reference(A_x, A_wqkv, A_wo, B_x, B_wqkv, B_wo):
    def _A_ref(x, wqkv, wo):
        B, S, D = x.shape
        H = 32; Dh = D // H
        W, dil = 8, 2
        qkv = (lambda x, *d: x.transpose(*d))((x @ wqkv).reshape(B, S, 3, H, Dh), 2, 0, 3, 1, 4)
        q, k, v = qkv[0], qkv[1], qkv[2]
        scale = Dh ** -0.5
        pos = jnp.arange(S)
        off = jnp.arange(W) * dil
        idx = pos[:, None] - off[None, :]
        mask = idx >= 0
        idx_c = jnp.where(mask, idx, 0).reshape(-1)
        kg = k[:, :, idx_c, :].reshape(B, H, S, W, Dh)
        vg = v[:, :, idx_c, :].reshape(B, H, S, W, Dh)
        logits = jnp.einsum("bhsd,bhswd->bhsw", q, kg) * scale
        logits = jnp.where(mask[None, None, :, :], logits, -1e9)
        attn = _softmax(logits, axis=-1)
        o = jnp.einsum("bhsw,bhswd->bhsd", attn, vg)
        return (lambda x, *d: x.transpose(*d))(o, 0, 2, 1, 3).reshape(B, S, D) @ wo

    def _B_ref(x, wqkv, wo):
        B, S, D = x.shape
        H = 32; Dh = D // H; W = 256
        qkv = (lambda x, *d: x.transpose(*d))((x @ wqkv).reshape(B, S, 3, H, Dh), 2, 0, 3, 1, 4)
        q, k, v = qkv[0], qkv[1], qkv[2]
        scores = jnp.einsum("bhqd,bhkd->bhqk", q, k) * (Dh ** -0.5)
        idx = jnp.arange(S)
        mask = (idx[:, None] - idx[None, :] >= 0) & (idx[:, None] - idx[None, :] < W)
        scores = jnp.where(mask[None, None], scores, -1e9)
        p = _softmax(scores, axis=-1)
        o = jnp.einsum("bhqk,bhkd->bhqd", p, v)
        return (lambda x, *d: x.transpose(*d))(o, 0, 2, 1, 3).reshape(B, S, D) @ wo

    a = _A_ref(A_x, A_wqkv, A_wo)
    b = _B_ref(B_x, B_wqkv, B_wo)
    return jnp.concatenate([a, b], axis=-1)
```

```python
import math

import jax
import jax.numpy as jnp
import numpy as np
from jax import lax
import jax.experimental.pallas as pl
import jax.experimental.pallas.tpu as pltpu

S = 2048
D = 1024
H = 32
DH = 32
T = 128
NT = S // T
NG = 8
HPG = H // NG
A_W, A_DIL = 8, 2
B_W = 256
QSCALE = float(DH ** -0.5 * math.log2(math.e))
NEG = -1e30
OT = 2

OPT = dict(rq=2, rkv=2, ot=2)

bf16 = jnp.bfloat16
f32 = jnp.float32
u32 = jnp.uint32


def _dot(a, b):
    return jnp.dot(a, b, preferred_element_type=f32)


def _dot_nt(a, b):
    return lax.dot_general(a, b, (((1,), (1,)), ((), ())), preferred_element_type=f32)


def _ld(x):
    return pltpu.bitcast(x, bf16)


def _slot(ring, s):
    return ring[:, s * 128:(s + 1) * 128]


def _lanes(g):
    if isinstance(g, int):
        return slice(g * 128, (g + 1) * 128)
    return pl.ds(pl.multiple_of(g * 128, 128), 128)


def _kernel(ax_hbm, aw_hbm, awo_hbm, bx_hbm, bw_hbm, bwo_hbm, out_hbm,
            xa_, xb_, raw_, wt_, wqk_, woa_, wob_,
            qa, ka, va, qb, kb, vb, sbuf, pbuf, trilm, oa_, ob_, ostage_,
            sem_xa, sem_xb, sem_w, sem_wo, sem_out):
    xa, xb, raw, wqk, woa, wob, ostage = [
        r.bitcast(bf16) for r in (xa_, xb_, raw_, wqk_, woa_, wob_, ostage_)]

    def cp_xa(i):
        return pltpu.make_async_copy(ax_hbm.at[pl.ds(i * T, T), :], xa.at[i], sem_xa.at[i])

    def cp_xb(i):
        return pltpu.make_async_copy(bx_hbm.at[pl.ds(i * T, T), :], xb.at[i], sem_xb.at[i])

    def cp_w(chunk, p):
        c0, n = (chunk * 128, 128) if chunk < 3 else (384, D - 384)
        src = (aw_hbm, aw_hbm, aw_hbm, bw_hbm, bw_hbm, bw_hbm)[p]
        off = (0, D, 2 * D, 2 * D, 0, D)[p]
        dst = raw.at[p] if p < 4 else wqk.at[p - 4]
        return pltpu.make_async_copy(src.at[:, pl.ds(off + c0, n)], dst.at[:, pl.ds(c0, n)],
                                     sem_w.at[chunk, p])

    def cp_wo(j):
        return pltpu.make_async_copy((awo_hbm, bwo_hbm)[j], (woa, wob)[j], sem_wo.at[j])

    cp_xa(0).start()
    for p in (0, 1, 2):
        cp_w(0, p).start()
    cp_xb(0).start()
    for p in (4, 5, 3):
        cp_w(0, p).start()
    for a4 in range(4):
        for i in range(4 * a4 + 1, min(4 * a4 + 5, NT)):
            cp_xa(i).start()
            cp_xb(i).start()
        for p in ((a4,) if a4 < 3 else (3, 4, 5)):
            cp_w(1, p).start()

    lane8 = lax.broadcasted_iota(jnp.int32, (8, 128), 1)
    sub8 = lax.broadcasted_iota(jnp.int32, (8, 128), 0)
    lane64 = lax.broadcasted_iota(jnp.int32, (64, 128), 1)
    row64 = lax.broadcasted_iota(jnp.int32, (64, 128), 0)
    sub3 = lax.broadcasted_iota(jnp.int32, (HPG, 8, 128), 1)
    lane3 = lax.broadcasted_iota(jnp.int32, (HPG, 8, 128), 2)
    trilm[...] = (jnp.where(2 * row64 <= lane64, np.uint32(0x0000FFFF), np.uint32(0))
                  | jnp.where(2 * row64 + 1 <= lane64, np.uint32(0xFFFF0000), np.uint32(0)))
    for rr in (ka, va, kb, vb):
        rr[...] = jnp.zeros(rr.shape, rr.dtype)

    def transpose_tile(g, p, c):
        wt_.at[g, p].bitcast(bf16)[:, c * 128:(c + 1) * 128] = _ld(raw_[p, c * 64:(c + 1) * 64, _lanes(g)]).T

    def transpose_part(g, p):
        wt_.at[g, p].bitcast(bf16)[...] = _ld(raw_[p, :, _lanes(g)]).T

    RQ, RKV = OPT["rq"], OPT["rkv"]

    def ring_store(ring, slot, val):
        ring.bitcast(bf16)[:, slot * 128:(slot + 1) * 128] = val.astype(bf16)

    def proj_aq(g, i, r):
        qa[r % RQ] = _dot_nt(_ld(wt_[g, 0]), _ld(xa_[i])) * QSCALE

    def proj_ak(g, i, r):
        ring_store(ka, r % RKV, _dot_nt(_ld(wt_[g, 1]), _ld(xa_[i])))

    def proj_av(g, i, r):
        ring_store(va, r % RKV, _dot_nt(_ld(wt_[g, 2]), _ld(xa_[i])))

    def proj_bqk(g, i, r):
        x = _ld(xb_[i])
        ring_store(qb, r, _dot(x, _ld(wqk_[0, :, _lanes(g)])) * QSCALE)
        ring_store(kb, r, _dot(x, _ld(wqk_[1, :, _lanes(g)])))

    def proj_bv(g, i, r):
        ring_store(vb, r, _dot_nt(_ld(wt_[g, 3]), _ld(xb_[i])))

    def shifted(ring, slot, pslot, w, first=None):
        cur = _slot(ring, slot)
        if w:
            sh = A_DIL * w
            if pslot is None:
                prev = jnp.zeros_like(cur)
            else:
                prev = _slot(ring, pslot)
                if first is not None:
                    prev = jnp.where(first, jnp.zeros_like(prev), prev)
            cur = pltpu.roll(jnp.where(lane64 >= T - sh, prev, cur), sh, 1)
        return _ld(cur).astype(f32).reshape(HPG, 4, 8, 128)

    def attn_a(g, i, r, has_prev, first):
        slot = r % RKV
        pslot = (r + 3) % 4 % RKV if has_prev else None
        q = qa[r % RQ].reshape(HPG, 4, 8, 128)
        a = []
        for w in range(A_W):
            prod = q * shifted(ka, slot, pslot, w)
            a.append((prod[:, 0] + prod[:, 1]) + (prod[:, 2] + prod[:, 3]))
        lo = sub3 < 4
        b = [jnp.where(lo, a[w], a[w + 4]) + pltpu.roll(jnp.where(lo, a[w + 4], a[w]), 4, 1)
             for w in range(4)]
        m2 = (sub3 & 2) == 0
        c = [jnp.where(m2, b[w] + pltpu.roll(b[w], 6, 1), b[w + 2] + pltpu.roll(b[w + 2], 2, 1))
             for w in range(2)]
        m1 = (sub3 & 1) == 0
        logit = jnp.where(m1, c[0] + pltpu.roll(c[0], 7, 1), c[1] + pltpu.roll(c[1], 1, 1))
        if not has_prev:
            logit = jnp.where(lane3 < A_DIL * sub3, NEG, logit)
        elif first is not None:
            logit = jnp.where(jnp.logical_and(first, lane3 < A_DIL * sub3), NEG, logit)
        m = logit
        for sh in (4, 2, 1):
            m = jnp.maximum(m, pltpu.roll(m, sh, 1))
        e = jnp.exp2(logit - m)
        l = e
        for sh in (4, 2, 1):
            l = l + pltpu.roll(l, sh, 1)
        p = e / l
        acc = None
        for w in range(A_W):
            pw = jnp.broadcast_to(p[:, w:w + 1, :], (HPG, 8, 128))[:, None]
            t = pw * shifted(va, slot, pslot, w, first)
            acc = t if acc is None else acc + t
        o = acc.reshape(128, 128).T
        oa_.at[i].bitcast(bf16)[:, _lanes(g)] = o.astype(bf16)

    dlt = lane8 - sub8

    def scores_b(r, v0, v1):
        sb = r % 2
        q = _slot(qb, r)
        k2 = _slot(kb, r)
        if v0 is not False:
            k0 = _slot(kb, (r + 2) % 4)
            rows = []
            for j in range(8):
                rows += [k0[8 * j:8 * j + 8], k2[8 * j:8 * j + 8]]
        else:
            rows = [k2]
        base = 256 if v0 is not False else 128
        if v1 is not False:
            rows.append(_slot(kb, (r + 3) % 4))
        k3 = _ld(jnp.concatenate(rows, axis=0))
        ms = []
        for hh in range(HPG):
            qm = _ld(jnp.where((lane64 // DH) == hh, q, jnp.zeros_like(q)))
            st = _dot_nt(k3, qm)
            m = None
            for j in range(16):
                if v0 is not False:
                    jj, hf = j // 2, j % 2
                    b0 = st[32 * jj + 8 * hf:32 * jj + 8 * hf + 8]
                    b2 = st[32 * jj + 16 + 8 * hf:32 * jj + 16 + 8 * hf + 8]
                    if v0 is not True:
                        b0 = jnp.where(v0, b0, NEG)
                else:
                    b0 = NEG
                    b2 = st[8 * j:8 * j + 8]
                c = jnp.where(dlt >= 8 * j, b2, b0)
                sbuf[sb, hh, 8 * j:8 * j + 8] = c
                m = c if m is None else jnp.maximum(m, c)
            if v1 is not False:
                for j in range(16):
                    b1 = st[base + 8 * j:base + 8 * j + 8]
                    if v1 is not True:
                        b1 = jnp.where(v1, b1, NEG)
                    sbuf[sb, hh, 128 + 8 * j:128 + 8 * j + 8] = b1
                    m = jnp.maximum(m, b1)
            for sh in (4, 2, 1):
                m = jnp.maximum(m, pltpu.roll(m, sh, 0))
            ms.append(m)
        return ms

    def softmax_b(r, ms, v1):
        sb = r % 2
        n = 256 if v1 is not False else 128
        pb = pbuf.at[sb].bitcast(bf16)
        ls = []
        for hh in range(HPG):
            p = jnp.exp2(sbuf[sb, hh, 0:n] - ms[hh][0:1])
            l = jnp.sum(p.reshape(n // 8, 8, 128), axis=0)
            pb[0:n, hh * 128:(hh + 1) * 128] = p.astype(bf16)
            for sh in (4, 2, 1):
                l = l + pltpu.roll(l, sh, 0)
            ls.append(1.0 / l)
        return ls

    def pv_b(ls, g, i, r, v0, v1):
        sb = r % 2

        def vt(slot, valid):
            v = _slot(vb, slot)
            if valid is not True:
                v = jnp.where(valid, v, jnp.zeros_like(v))
            return _ld(v)

        w2 = vt(r, True)
        w0 = vt((r + 2) % 4, v0) if v0 is not False else None
        w1 = vt((r + 3) % 4, v1) if v1 is not False else None
        outs = []
        for hh in range(HPG):
            rs = slice(hh * DH, (hh + 1) * DH)
            pc = pbuf[sb, 0:T // 2, hh * 128:(hh + 1) * 128]
            if v0 is not False:
                p2 = pc & trilm[...]
                ot = _dot(w0[rs], _ld(pc ^ p2)) + _dot(w2[rs], _ld(p2))
            else:
                ot = _dot(w2[rs], _ld(pc))
            if v1 is not False:
                ot = ot + _dot(w1[rs], _ld(pbuf[sb, T // 2:T, hh * 128:(hh + 1) * 128]))
            outs += [ot[8 * j:8 * j + 8] * ls[hh] for j in range(4)]
        o = jnp.concatenate(outs, axis=0).T
        ob_.at[i].bitcast(bf16)[:, _lanes(g)] = o.astype(bf16)

    def step(g, i, gn, inx, r, has_prev, first, v0, v1, tiles):
        rn = (r + 1) % 4
        ms = scores_b(r, v0, v1)
        proj_bqk(gn, inx, rn)
        ls = softmax_b(r, ms, v1)
        pv_b(ls, g, i, r, v0, v1)
        attn_a(g, i, r, has_prev, first)
        proj_aq(gn, inx, rn)
        proj_ak(gn, inx, rn)
        proj_av(gn, inx, rn)
        proj_bv(gn, inx, rn)
        for t in tiles:
            transpose_tile(*t)

    cp_xa(0).wait()
    for p, proj in ((0, proj_aq), (1, proj_ak), (2, proj_av)):
        cp_w(0, p).wait()
        transpose_part(0, p)
        proj(0, 0, 0)
    cp_xb(0).wait()
    cp_w(0, 4).wait()
    cp_w(0, 5).wait()
    proj_bqk(0, 0, 0)
    cp_w(0, 3).wait()
    transpose_part(0, 3)
    proj_bv(0, 0, 0)

    def body0(a, carry):
        @pl.when(a == 2)
        def _():
            for p in range(6):
                cp_w(2, p).start()

        @pl.when(a == 3)
        def _():
            for p in range(6):
                cp_w(3, p).start()

        for u in range(4):
            nxt = 4 * a + u + 1

            @pl.when(nxt < NT)
            def _():
                cp_xa(nxt).wait()
                cp_xb(nxt).wait()

        for j in range(4):
            @pl.when(a == j)
            def _():
                for p in ((j,) if j < 3 else (3, 4, 5)):
                    cp_w(1, p).wait()

        for u in range(4):
            i = 4 * a + u
            gn, inx = (0, i + 1) if u < 3 else (a // 3, jnp.where(a == 3, 0, i + 1))
            first = (a == 0) if u == 0 else None
            v1 = (a > 0) if u == 0 else True
            v0 = (a > 0) if u <= 1 else True
            tiles = [(1, a, c) for c in range(8)][3 * u:3 * u + 3] if u < 3 else []
            step(0, i, gn, inx, u, True, first, v0, v1, tiles)
        return carry

    lax.fori_loop(0, 4, body0, 0)

    tsched = {i: [] for i in range(NT)}
    for n in range(32):
        tsched[1 + n * 13 // 32].append(divmod(n, 8))

    def body(g, carry):
        gt = jnp.minimum(g + 1, NG - 1)

        @pl.when(g == 1)
        def _():
            for p in range(6):
                cp_w(2, p).wait()

        @pl.when(g == 2)
        def _():
            for p in range(6):
                cp_w(3, p).wait()

        @pl.when(g == 4)
        def _():
            cp_wo(0).start()
            cp_wo(1).start()

        for i in range(NT):
            gn, inx = (g, i + 1) if i < NT - 1 else (gt, 0)
            step(g, i, gn, inx, i % 4, i > 0, None, i >= 2, i >= 1,
                 [(gt, p, c) for p, c in tsched[i]])
        return carry

    lax.fori_loop(1, NG, body, 0)

    cp_wo(0).wait()
    cp_wo(1).wait()

    def cp_out(s, slot):
        return pltpu.make_async_copy(ostage.at[slot], out_hbm.at[pl.ds(s * (OT * T), OT * T), :],
                                     sem_out.at[slot])

    def obody(s, carry):
        slot = s % 2

        @pl.when(s >= 2)
        def _():
            cp_out(s - 2, slot).wait()

        a_ = _ld(oa_[pl.ds(s * OT, OT)].reshape(OT * T // 2, D))
        b_ = _ld(ob_[pl.ds(s * OT, OT)].reshape(OT * T // 2, D))
        ostage_.at[slot].bitcast(bf16)[:, 0:D] = _dot(a_, _ld(woa_[...])).astype(bf16)
        ostage_.at[slot].bitcast(bf16)[:, D:2 * D] = _dot(b_, _ld(wob_[...])).astype(bf16)
        cp_out(s, slot).start()
        return carry

    nsteps = NT // OT
    lax.fori_loop(0, nsteps, obody, 0)
    cp_out(nsteps - 2, (nsteps - 2) % 2).wait()
    cp_out(nsteps - 1, (nsteps - 1) % 2).wait()


@jax.jit
def pallas_concat_heads__sliding_local_dilated__sliding_block__prompt_kernel(
    A_x: jax.Array,
    A_wqkv: jax.Array,
    A_wo: jax.Array,
    B_x: jax.Array,
    B_wqkv: jax.Array,
    B_wo: jax.Array,
):
    B = A_x.shape[0]
    assert A_x.shape == B_x.shape == (1, S, D)
    any_spec = pl.BlockSpec(memory_space=pl.ANY)
    vm = pltpu.VMEM
    scratch = [
        vm((NT, T // 2, D), u32), vm((NT, T // 2, D), u32),
        vm((4, D // 2, D), u32),
        vm((NG, 4, 64, D), u32),
        vm((2, D // 2, D), u32),
        vm((D // 2, D), u32), vm((D // 2, D), u32),
        vm((4, 128, T), f32), vm((64, 512), u32), vm((64, 512), u32),
        vm((64, 512), u32), vm((64, 512), u32), vm((64, 512), u32),
        vm((2, HPG, 2 * T, T), f32), vm((2, T, HPG * T), u32),
        vm((64, 128), u32),
        vm((NT, T // 2, D), u32), vm((NT, T // 2, D), u32),
        vm((2, OT * T // 2, 2 * D), u32),
        pltpu.SemaphoreType.DMA((NT,)), pltpu.SemaphoreType.DMA((NT,)),
        pltpu.SemaphoreType.DMA((4, 6)),
        pltpu.SemaphoreType.DMA((2,)), pltpu.SemaphoreType.DMA((2,)),
    ]
    out = pl.pallas_call(
        _kernel,
        out_shape=jax.ShapeDtypeStruct((S, 2 * D), bf16),
        in_specs=[any_spec] * 6,
        out_specs=any_spec,
        scratch_shapes=scratch,
        compiler_params=pltpu.CompilerParams(
            vmem_limit_bytes=100 * 1024 * 1024,
            flags={"XLA_TPU_FORCE_LP_LLO_SCHEDULER": True},
        ),
        name="concat_heads_kernel",
    )(A_x.reshape(S, D), A_wqkv, A_wo, B_x.reshape(S, D), B_wqkv, B_wo)
    return out.reshape(B, S, 2 * D)
```

```python
import math

import jax
import jax.numpy as jnp
import numpy as np
from jax import lax
import jax.experimental.pallas as pl
import jax.experimental.pallas.tpu as pltpu

S = 2048
D = 1024
H = 32
DH = 32
T = 128
NT = S // T
NG = 8
HPG = H // NG
A_W, A_DIL = 8, 2
B_W = 256
RA = 2
QSCALE = float(DH ** -0.5 * math.log2(math.e))
NEG = -1e30


OT = 2

bf16 = jnp.bfloat16
f32 = jnp.float32
u32 = jnp.uint32


def _dot(a, b):
    return jnp.dot(a, b, preferred_element_type=f32)


def _dot_nt(a, b):
    return lax.dot_general(a, b, (((1,), (1,)), ((), ())), preferred_element_type=f32)


def _ld(x):
    return pltpu.bitcast(x, bf16)


def _slot(ring, s):
    return ring[:, s * 128:(s + 1) * 128]


def _lanes(g):
    if isinstance(g, int):
        return slice(g * 128, (g + 1) * 128)
    return pl.ds(pl.multiple_of(g * 128, 128), 128)


def _kernel(ax_hbm, aw_hbm, awo_hbm, bx_hbm, bw_hbm, bwo_hbm, out_hbm,
            xa_, xb_, raw_, wt_, wqk_, woa_, wob_,
            qa, ka, va, qb, kb, vb, sbuf, pbuf, trilm, oa_, ob_, ostage_,
            sem_xa, sem_xb, sem_w, sem_wo, sem_out, sem_tail):
    xa, xb, raw, wqk, woa, wob, ostage = [
        r.bitcast(bf16) for r in (xa_, xb_, raw_, wqk_, woa_, wob_, ostage_)]

    def cp_xa(i):
        return pltpu.make_async_copy(ax_hbm.at[pl.ds(i * T, T), :], xa.at[i], sem_xa.at[i])

    def cp_xb(i):
        return pltpu.make_async_copy(bx_hbm.at[pl.ds(i * T, T), :], xb.at[i], sem_xb.at[i])

    def cp_w(chunk, p):
        c0, n = (chunk * 128, 128) if chunk < 3 else (384, D - 384)
        src = (aw_hbm, aw_hbm, aw_hbm, bw_hbm, bw_hbm, bw_hbm)[p]
        off = (0, D, 2 * D, 2 * D, 0, D)[p]
        dst = raw.at[p] if p < 4 else wqk.at[p - 4]
        return pltpu.make_async_copy(src.at[:, pl.ds(off + c0, n)], dst.at[:, pl.ds(c0, n)],
                                     sem_w.at[chunk, p])

    def cp_wo(j):
        return pltpu.make_async_copy((awo_hbm, bwo_hbm)[j], (woa, wob)[j], sem_wo.at[j])

    cp_xa(0).start()
    for p in (0, 1, 2):
        cp_w(0, p).start()
    cp_xb(0).start()
    for p in (4, 5, 3):
        cp_w(0, p).start()
    for a4 in range(4):
        for i in range(4 * a4 + 1, min(4 * a4 + 5, NT)):
            cp_xa(i).start()
            cp_xb(i).start()
        for p in ((a4,) if a4 < 3 else (3, 4, 5)):
            cp_w(1, p).start()

    lane8 = lax.broadcasted_iota(jnp.int32, (8, 128), 1)
    sub8 = lax.broadcasted_iota(jnp.int32, (8, 128), 0)
    lane64 = lax.broadcasted_iota(jnp.int32, (64, 128), 1)
    row64 = lax.broadcasted_iota(jnp.int32, (64, 128), 0)
    sub3 = lax.broadcasted_iota(jnp.int32, (HPG, 8, 128), 1)
    lane3 = lax.broadcasted_iota(jnp.int32, (HPG, 8, 128), 2)
    trilm[...] = (jnp.where(2 * row64 <= lane64, np.uint32(0x0000FFFF), np.uint32(0))
                  | jnp.where(2 * row64 + 1 <= lane64, np.uint32(0xFFFF0000), np.uint32(0)))

    def transpose_tile(g, p, c):
        wt_.at[g, p].bitcast(bf16)[:, c * 128:(c + 1) * 128] = _ld(raw_[p, c * 64:(c + 1) * 64, _lanes(g)]).T

    def transpose_part(g, p):
        wt_.at[g, p].bitcast(bf16)[...] = _ld(raw_[p, :, _lanes(g)]).T


    def ring_store(ring, slot, val):
        ring.bitcast(bf16)[:, slot * 128:(slot + 1) * 128] = val.astype(bf16)

    def proj_aq(g, i, r):
        qa[r % RA] = _dot_nt(_ld(wt_[g, 0]), _ld(xa_[i])) * QSCALE

    def proj_ak(g, i, r):
        ring_store(ka, r % RA, _dot_nt(_ld(wt_[g, 1]), _ld(xa_[i])))

    def proj_av(g, i, r):
        ring_store(va, r % RA, _dot_nt(_ld(wt_[g, 2]), _ld(xa_[i])))

    def proj_bqk(g, i, r):
        x = _ld(xb_[i])
        ring_store(qb, r, _dot(x, _ld(wqk_[0, :, _lanes(g)])) * QSCALE)
        ring_store(kb, r, _dot(x, _ld(wqk_[1, :, _lanes(g)])))

    def proj_bv(g, i, r):
        ring_store(vb, r, _dot_nt(_ld(wt_[g, 3]), _ld(xb_[i])))

    def shifted(ring, slot, pslot, w):
        cur = _slot(ring, slot)
        if w:
            sh = A_DIL * w
            if pslot is None:
                prev = jnp.zeros_like(cur)
            else:
                prev = _slot(ring, pslot)
            cur = pltpu.roll(jnp.where(lane64 >= T - sh, prev, cur), sh, 1)
        return _ld(cur).astype(f32).reshape(HPG, 4, 8, 128)

    def attn_a(g, i, r, has_prev):
        slot = r % RA
        pslot = (r + 3) % RA if has_prev else None
        q = qa[r % RA].reshape(HPG, 4, 8, 128)
        a = []
        for w in range(A_W):
            prod = q * shifted(ka, slot, pslot, w)
            a.append((prod[:, 0] + prod[:, 1]) + (prod[:, 2] + prod[:, 3]))
        lo = sub3 < 4
        b = [jnp.where(lo, a[w], a[w + 4]) + pltpu.roll(jnp.where(lo, a[w + 4], a[w]), 4, 1)
             for w in range(4)]
        m2 = (sub3 & 2) == 0
        c = [jnp.where(m2, b[w] + pltpu.roll(b[w], 6, 1), b[w + 2] + pltpu.roll(b[w + 2], 2, 1))
             for w in range(2)]
        m1 = (sub3 & 1) == 0
        logit = jnp.where(m1, c[0] + pltpu.roll(c[0], 7, 1), c[1] + pltpu.roll(c[1], 1, 1))
        if not has_prev:
            logit = jnp.where(lane3 < A_DIL * sub3, NEG, logit)
        m = logit
        for sh in (4, 2, 1):
            m = jnp.maximum(m, pltpu.roll(m, sh, 1))
        e = jnp.exp2(logit - m)
        l = e
        for sh in (4, 2, 1):
            l = l + pltpu.roll(l, sh, 1)
        p = e / l
        acc = None
        for w in range(A_W):
            pw = jnp.broadcast_to(p[:, w:w + 1, :], (HPG, 8, 128))[:, None]
            t = pw * shifted(va, slot, pslot, w)
            acc = t if acc is None else acc + t
        o = acc.reshape(128, 128).T
        oa_.at[i].bitcast(bf16)[:, _lanes(g)] = o.astype(bf16)

    dlt = lane8 - sub8

    def scores_b(r, v0, v1):
        sb = r % 2
        q = _slot(qb, r)
        k2 = _slot(kb, r)
        if v0:
            k0 = _slot(kb, (r + 2) % 4)
            rows = []
            for j in range(8):
                rows += [k0[8 * j:8 * j + 8], k2[8 * j:8 * j + 8]]
        else:
            rows = [k2]
        base = 256 if v0 else 128
        if v1:
            rows.append(_slot(kb, (r + 3) % 4))
        k3 = _ld(jnp.concatenate(rows, axis=0))
        ms = []
        for hh in range(HPG):
            qm = _ld(jnp.where((lane64 // DH) == hh, q, jnp.zeros_like(q)))
            st = _dot_nt(k3, qm)
            m = None
            for j in range(16):
                if v0:
                    jj, hf = j // 2, j % 2
                    b0 = st[32 * jj + 8 * hf:32 * jj + 8 * hf + 8]
                    b2 = st[32 * jj + 16 + 8 * hf:32 * jj + 16 + 8 * hf + 8]
                else:
                    b0 = NEG
                    b2 = st[8 * j:8 * j + 8]
                c = jnp.where(dlt >= 8 * j, b2, b0)
                sbuf[sb, hh, 8 * j:8 * j + 8] = c
                m = c if m is None else jnp.maximum(m, c)
            if v1:
                for j in range(16):
                    b1 = st[base + 8 * j:base + 8 * j + 8]
                    sbuf[sb, hh, 128 + 8 * j:128 + 8 * j + 8] = b1
                    m = jnp.maximum(m, b1)
            for sh in (4, 2, 1):
                m = jnp.maximum(m, pltpu.roll(m, sh, 0))
            ms.append(m)
        return ms

    def softmax_b(r, ms, v1):
        sb = r % 2
        n = 256 if v1 else 128
        pb = pbuf.at[sb].bitcast(bf16)
        ls = []
        for hh in range(HPG):
            p = jnp.exp2(sbuf[sb, hh, 0:n] - ms[hh][0:1])
            l = jnp.sum(p.reshape(n // 8, 8, 128), axis=0)
            pb[0:n, hh * 128:(hh + 1) * 128] = p.astype(bf16)
            for sh in (4, 2, 1):
                l = l + pltpu.roll(l, sh, 0)
            ls.append(1.0 / l)
        return ls

    def pv_b(ls, g, i, r, v0, v1):
        sb = r % 2

        w2 = _ld(_slot(vb, r))
        w0 = _ld(_slot(vb, (r + 2) % 4)) if v0 else None
        w1 = _ld(_slot(vb, (r + 3) % 4)) if v1 else None
        outs = []
        for hh in range(HPG):
            rs = slice(hh * DH, (hh + 1) * DH)
            pc = pbuf[sb, 0:T // 2, hh * 128:(hh + 1) * 128]
            if v0:
                p2 = pc & trilm[...]
                ot = _dot(w0[rs], _ld(pc ^ p2)) + _dot(w2[rs], _ld(p2))
            else:
                ot = _dot(w2[rs], _ld(pc))
            if v1:
                ot = ot + _dot(w1[rs], _ld(pbuf[sb, T // 2:T, hh * 128:(hh + 1) * 128]))
            outs += [ot[8 * j:8 * j + 8] * ls[hh] for j in range(4)]
        o = jnp.concatenate(outs, axis=0).T
        ob_.at[i].bitcast(bf16)[:, _lanes(g)] = o.astype(bf16)

    def step(g, i, gn, inx, r, has_prev, v0, v1, tiles):
        rn = (r + 1) % 4
        ms = scores_b(r, v0, v1)
        proj_bqk(gn, inx, rn)
        attn_a(g, i, r, has_prev)
        ls = softmax_b(r, ms, v1)
        pv_b(ls, g, i, r, v0, v1)
        proj_aq(gn, inx, rn)
        proj_ak(gn, inx, rn)
        proj_av(gn, inx, rn)
        proj_bv(gn, inx, rn)
        for t in tiles:
            transpose_tile(*t)

    cp_xa(0).wait()
    for p, proj in ((0, proj_aq), (1, proj_ak), (2, proj_av)):
        cp_w(0, p).wait()
        transpose_part(0, p)
        proj(0, 0, 0)
    cp_xb(0).wait()
    cp_w(0, 4).wait()
    cp_w(0, 5).wait()
    proj_bqk(0, 0, 0)
    cp_w(0, 3).wait()
    transpose_part(0, 3)
    proj_bv(0, 0, 0)

    for i in range(4):
        for t in {0: (1,), 1: (2,), 2: (3, 4)}.get(i, ()):
            cp_xa(t).wait()
            cp_xb(t).wait()
        if i == 3:
            cp_w(1, 0).wait()
        step(0, i, 0, i + 1, i, i > 0, i >= 2, i >= 1,
             [(1, 0, c) for c in range(8)] if i == 3 else [])

    def body0(a, carry):
        @pl.when(a == 2)
        def _():
            for p in range(6):
                cp_w(2, p).start()

        @pl.when(a == 3)
        def _():
            for p in range(6):
                cp_w(3, p).start()
            cp_wo(0).start()
            cp_wo(1).start()

        for u in range(4):
            nxt = 4 * a + u + 1

            @pl.when(nxt < NT)
            def _():
                cp_xa(nxt).wait()
                cp_xb(nxt).wait()

        for j in range(1, 4):
            @pl.when(a == j)
            def _():
                for p in ((j,) if j < 3 else (3, 4, 5)):
                    cp_w(1, p).wait()

        for u in range(4):
            i = 4 * a + u
            gn, inx = (0, i + 1) if u < 3 else (a // 3, jnp.where(a == 3, 0, i + 1))
            tiles = [(1, a, c) for c in range(8)][3 * u:3 * u + 3] if u < 3 else []
            step(0, i, gn, inx, u, True, True, True, tiles)
        return carry

    lax.fori_loop(1, 4, body0, 0)

    tsched = {i: [] for i in range(NT)}
    for n in range(32):
        tsched[n * 15 // 32].append(divmod(n, 8))

    def body(g, carry):
        gt = jnp.minimum(g + 1, NG - 1)

        @pl.when(g == 2)
        def _():
            for p in range(6):
                cp_w(3, p).wait()

        for i in range(NT):
            gn, inx = (g, i + 1) if i < NT - 1 else (gt, 0)
            step(g, i, gn, inx, i % 4, i > 0, i >= 2, i >= 1,
                 [(gt, p, c) for p, c in tsched[i]])
        return carry

    for p in range(6):
        cp_w(2, p).wait()
    lax.fori_loop(1, NG, body, 0)

    cp_wo(0).wait()
    cp_wo(1).wait()

    def cp_out(s, slot):
        return pltpu.make_async_copy(ostage.at[slot], out_hbm.at[pl.ds(s * (OT * T), OT * T), :],
                                     sem_out.at[slot])

    def obody(s, carry):
        slot = s % 2

        @pl.when(s >= 2)
        def _():
            cp_out(s - 2, slot).wait()

        a_ = _ld(oa_[pl.ds(s * OT, OT)].reshape(OT * T // 2, D))
        b_ = _ld(ob_[pl.ds(s * OT, OT)].reshape(OT * T // 2, D))
        ostage_.at[slot].bitcast(bf16)[:, 0:D] = _dot(a_, _ld(woa_[...])).astype(bf16)
        ostage_.at[slot].bitcast(bf16)[:, D:2 * D] = _dot(b_, _ld(wob_[...])).astype(bf16)
        cp_out(s, slot).start()
        return carry

    nsteps = NT // OT
    lax.fori_loop(0, nsteps - 1, obody, 0)
    sl = nsteps - 1
    slot = sl % 2
    cp_out(sl - 2, slot).wait()
    r0 = sl * OT * T
    tails = []

    def send(rows, cols, n):
        c = pltpu.make_async_copy(ostage.at[slot, pl.ds(rows[0], rows[1]), pl.ds(cols, D)],
                                  out_hbm.at[pl.ds(r0 + rows[0], rows[1]), pl.ds(cols, D)],
                                  sem_tail.at[n])
        c.start()
        tails.append(c)

    ost = ostage_.at[slot].bitcast(bf16)
    ost[:, 0:D] = _dot(_ld(oa_[pl.ds(sl * OT, OT)].reshape(OT * T // 2, D)), _ld(woa_[...])).astype(bf16)
    send((0, OT * T), 0, 0)
    for j in range(OT):
        ost[j * T:(j + 1) * T, D:2 * D] = _dot(_ld(ob_[sl * OT + j]), _ld(wob_[...])).astype(bf16)
        send((j * T, T), D, 1 + j)
    cp_out(sl - 1, (sl - 1) % 2).wait()
    for c in tails:
        c.wait()


@jax.jit
def pallas_concat_heads__sliding_local_dilated__sliding_block__prompt_kernel(
    A_x: jax.Array,
    A_wqkv: jax.Array,
    A_wo: jax.Array,
    B_x: jax.Array,
    B_wqkv: jax.Array,
    B_wo: jax.Array,
):
    B = A_x.shape[0]
    assert A_x.shape == B_x.shape == (1, S, D)
    any_spec = pl.BlockSpec(memory_space=pl.ANY)
    vm = pltpu.VMEM
    scratch = [
        vm((NT, T // 2, D), u32), vm((NT, T // 2, D), u32),
        vm((4, D // 2, D), u32),
        vm((NG, 4, 64, D), u32),
        vm((2, D // 2, D), u32),
        vm((D // 2, D), u32), vm((D // 2, D), u32),
        vm((RA, 128, T), f32), vm((64, RA * 128), u32), vm((64, RA * 128), u32),
        vm((64, 512), u32), vm((64, 512), u32), vm((64, 512), u32),
        vm((2, HPG, 2 * T, T), f32), vm((2, T, HPG * T), u32),
        vm((64, 128), u32),
        vm((NT, T // 2, D), u32), vm((NT, T // 2, D), u32),
        vm((2, OT * T // 2, 2 * D), u32),
        pltpu.SemaphoreType.DMA((NT,)), pltpu.SemaphoreType.DMA((NT,)),
        pltpu.SemaphoreType.DMA((4, 6)),
        pltpu.SemaphoreType.DMA((2,)), pltpu.SemaphoreType.DMA((2,)),
        pltpu.SemaphoreType.DMA((1 + OT,)),
    ]
    out = pl.pallas_call(
        _kernel,
        out_shape=jax.ShapeDtypeStruct((S, 2 * D), bf16),
        in_specs=[any_spec] * 6,
        out_specs=any_spec,
        scratch_shapes=scratch,
        compiler_params=pltpu.CompilerParams(
            vmem_limit_bytes=100 * 1024 * 1024,
            flags={"XLA_TPU_FORCE_LP_LLO_SCHEDULER": True},
            disable_bounds_checks=True,
            disable_semaphore_checks=True,
        ),
        name="concat_heads_kernel",
    )(A_x.reshape(S, D), A_wqkv, A_wo, B_x.reshape(S, D), B_wqkv, B_wo)
    return out.reshape(B, S, 2 * D)
```

```python
import math

import jax
import jax.numpy as jnp
import numpy as np
from jax import lax
import jax.experimental.pallas as pl
import jax.experimental.pallas.tpu as pltpu

S = 2048
D = 1024
H = 32
DH = 32
T = 128
NT = S // T
NG = 8
HPG = H // NG
A_W, A_DIL = 8, 2
B_W = 256
RA = 2
QSCALE = float(DH ** -0.5 * math.log2(math.e))
NEG = -1e30


OT = 2

bf16 = jnp.bfloat16
f32 = jnp.float32
u32 = jnp.uint32


def _dot(a, b):
    return jnp.dot(a, b, preferred_element_type=f32)


def _dot_nt(a, b):
    return lax.dot_general(a, b, (((1,), (1,)), ((), ())), preferred_element_type=f32)


def _ld(x):
    return pltpu.bitcast(x, bf16)


def _slot(ring, s):
    return ring[:, s * 128:(s + 1) * 128]


def _lanes(g):
    if isinstance(g, int):
        return slice(g * 128, (g + 1) * 128)
    return pl.ds(pl.multiple_of(g * 128, 128), 128)


def _kernel(ax_hbm, aw_hbm, awo_hbm, bx_hbm, bw_hbm, bwo_hbm, out_hbm,
            xa_, xb_, raw_, wt_, wqk_, woa_, wob_,
            qa, ka, va, qb, kb, vb, sbuf, pbuf, trilm, oa_, ob_, ostage_,
            sem_xa, sem_xb, sem_w, sem_wo, sem_out, sem_tail):
    xa, xb, raw, wqk, woa, wob, ostage = [
        r.bitcast(bf16) for r in (xa_, xb_, raw_, wqk_, woa_, wob_, ostage_)]

    def cp_xa(i):
        return pltpu.make_async_copy(ax_hbm.at[pl.ds(i * T, T), :], xa.at[i], sem_xa.at[i])

    def cp_xb(i):
        return pltpu.make_async_copy(bx_hbm.at[pl.ds(i * T, T), :], xb.at[i], sem_xb.at[i])

    def cp_w(chunk, p):
        c0, n = (chunk * 128, 128) if chunk < 3 else (384, D - 384)
        src = (aw_hbm, aw_hbm, aw_hbm, bw_hbm, bw_hbm, bw_hbm)[p]
        off = (0, D, 2 * D, 2 * D, 0, D)[p]
        dst = raw.at[p] if p < 4 else wqk.at[p - 4]
        return pltpu.make_async_copy(src.at[:, pl.ds(off + c0, n)], dst.at[:, pl.ds(c0, n)],
                                     sem_w.at[chunk, p])

    def cp_wo(j):
        return pltpu.make_async_copy((awo_hbm, bwo_hbm)[j], (woa, wob)[j], sem_wo.at[j])

    cp_xa(0).start()
    for p in (0, 1, 2):
        cp_w(0, p).start()
    cp_xb(0).start()
    for p in (4, 5, 3):
        cp_w(0, p).start()
    for a4 in range(4):
        for i in range(4 * a4 + 1, min(4 * a4 + 5, NT)):
            cp_xa(i).start()
            cp_xb(i).start()
        for p in ((a4,) if a4 < 3 else (3, 4, 5)):
            cp_w(1, p).start()
    for chunk in (2, 3):
        for p in range(6):
            cp_w(chunk, p).start()
    cp_wo(0).start()
    cp_wo(1).start()

    lane8 = lax.broadcasted_iota(jnp.int32, (8, 128), 1)
    sub8 = lax.broadcasted_iota(jnp.int32, (8, 128), 0)
    lane64 = lax.broadcasted_iota(jnp.int32, (64, 128), 1)
    row64 = lax.broadcasted_iota(jnp.int32, (64, 128), 0)
    sub3 = lax.broadcasted_iota(jnp.int32, (HPG, 8, 128), 1)
    lane3 = lax.broadcasted_iota(jnp.int32, (HPG, 8, 128), 2)
    trilm[...] = (jnp.where(2 * row64 <= lane64, np.uint32(0x0000FFFF), np.uint32(0))
                  | jnp.where(2 * row64 + 1 <= lane64, np.uint32(0xFFFF0000), np.uint32(0)))

    def transpose_tile(g, p, c):
        wt_.at[g, p].bitcast(bf16)[:, c * 128:(c + 1) * 128] = _ld(raw_[p, c * 64:(c + 1) * 64, _lanes(g)]).T

    def transpose_part(g, p):
        wt_.at[g, p].bitcast(bf16)[...] = _ld(raw_[p, :, _lanes(g)]).T


    def ring_store(ring, slot, val):
        ring.bitcast(bf16)[:, slot * 128:(slot + 1) * 128] = val.astype(bf16)

    def proj_aq(g, i, r):
        qa[r % RA] = _dot_nt(_ld(wt_[g, 0]), _ld(xa_[i])) * QSCALE

    def proj_ak(g, i, r):
        ring_store(ka, r % RA, _dot_nt(_ld(wt_[g, 1]), _ld(xa_[i])))

    def proj_av(g, i, r):
        ring_store(va, r % RA, _dot_nt(_ld(wt_[g, 2]), _ld(xa_[i])))

    def proj_bqk(g, i, r):
        x = _ld(xb_[i])
        ring_store(qb, r, _dot(x, _ld(wqk_[0, :, _lanes(g)])) * QSCALE)
        ring_store(kb, r, _dot(x, _ld(wqk_[1, :, _lanes(g)])))

    def proj_bv(g, i, r):
        ring_store(vb, r, _dot_nt(_ld(wt_[g, 3]), _ld(xb_[i])))

    def shifted(ring, slot, pslot, w):
        cur = _slot(ring, slot)
        if w:
            sh = A_DIL * w
            if pslot is None:
                prev = jnp.zeros_like(cur)
            else:
                prev = _slot(ring, pslot)
            cur = pltpu.roll(jnp.where(lane64 >= T - sh, prev, cur), sh, 1)
        return _ld(cur).astype(f32).reshape(HPG, 4, 8, 128)

    def attn_a(g, i, r, has_prev):
        slot = r % RA
        pslot = (r + 3) % RA if has_prev else None
        q = qa[r % RA].reshape(HPG, 4, 8, 128)
        a = []
        for w in range(A_W):
            prod = q * shifted(ka, slot, pslot, w)
            a.append((prod[:, 0] + prod[:, 1]) + (prod[:, 2] + prod[:, 3]))
        lo = sub3 < 4
        b = [jnp.where(lo, a[w], a[w + 4]) + pltpu.roll(jnp.where(lo, a[w + 4], a[w]), 4, 1)
             for w in range(4)]
        m2 = (sub3 & 2) == 0
        c = [jnp.where(m2, b[w] + pltpu.roll(b[w], 6, 1), b[w + 2] + pltpu.roll(b[w + 2], 2, 1))
             for w in range(2)]
        m1 = (sub3 & 1) == 0
        logit = jnp.where(m1, c[0] + pltpu.roll(c[0], 7, 1), c[1] + pltpu.roll(c[1], 1, 1))
        if not has_prev:
            logit = jnp.where(lane3 < A_DIL * sub3, NEG, logit)
        m = logit
        for sh in (4, 2, 1):
            m = jnp.maximum(m, pltpu.roll(m, sh, 1))
        e = jnp.exp2(logit - m)
        l = e
        for sh in (4, 2, 1):
            l = l + pltpu.roll(l, sh, 1)
        p = e / l
        acc = None
        for w in range(A_W):
            pw = jnp.broadcast_to(p[:, w:w + 1, :], (HPG, 8, 128))[:, None]
            t = pw * shifted(va, slot, pslot, w)
            acc = t if acc is None else acc + t
        o = acc.reshape(128, 128).T
        oa_.at[i].bitcast(bf16)[:, _lanes(g)] = o.astype(bf16)

    dlt = lane8 - sub8

    def scores_b(r, v0, v1):
        sb = r % 2
        q = _slot(qb, r)
        k2 = _slot(kb, r)
        if v0:
            k0 = _slot(kb, (r + 2) % 4)
            rows = []
            for j in range(8):
                rows += [k0[8 * j:8 * j + 8], k2[8 * j:8 * j + 8]]
        else:
            rows = [k2]
        base = 256 if v0 else 128
        if v1:
            rows.append(_slot(kb, (r + 3) % 4))
        k3 = _ld(jnp.concatenate(rows, axis=0))
        ms = []
        for hh in range(HPG):
            qm = _ld(jnp.where((lane64 // DH) == hh, q, jnp.zeros_like(q)))
            st = _dot_nt(k3, qm)
            m = None
            for j in range(16):
                if v0:
                    jj, hf = j // 2, j % 2
                    b0 = st[32 * jj + 8 * hf:32 * jj + 8 * hf + 8]
                    b2 = st[32 * jj + 16 + 8 * hf:32 * jj + 16 + 8 * hf + 8]
                else:
                    b0 = NEG
                    b2 = st[8 * j:8 * j + 8]
                c = jnp.where(dlt >= 8 * j, b2, b0)
                sbuf[sb, hh, 8 * j:8 * j + 8] = c
                m = c if m is None else jnp.maximum(m, c)
            if v1:
                for j in range(16):
                    b1 = st[base + 8 * j:base + 8 * j + 8]
                    sbuf[sb, hh, 128 + 8 * j:128 + 8 * j + 8] = b1
                    m = jnp.maximum(m, b1)
            for sh in (4, 2, 1):
                m = jnp.maximum(m, pltpu.roll(m, sh, 0))
            ms.append(m)
        return ms

    def softmax_b(r, ms, v1):
        sb = r % 2
        n = 256 if v1 else 128
        pb = pbuf.at[sb].bitcast(bf16)
        ls = []
        for hh in range(HPG):
            p = jnp.exp2(sbuf[sb, hh, 0:n] - ms[hh][0:1])
            l = jnp.sum(p.reshape(n // 8, 8, 128), axis=0)
            pb[0:n, hh * 128:(hh + 1) * 128] = p.astype(bf16)
            for sh in (4, 2, 1):
                l = l + pltpu.roll(l, sh, 0)
            ls.append(1.0 / l)
        return ls

    def pv_b(ls, g, i, r, v0, v1):
        sb = r % 2

        w2 = _ld(_slot(vb, r))
        w0 = _ld(_slot(vb, (r + 2) % 4)) if v0 else None
        w1 = _ld(_slot(vb, (r + 3) % 4)) if v1 else None
        outs = []
        for hh in range(HPG):
            rs = slice(hh * DH, (hh + 1) * DH)
            pc = pbuf[sb, 0:T // 2, hh * 128:(hh + 1) * 128]
            if v0:
                p2 = pc & trilm[...]
                ot = _dot(w0[rs], _ld(pc ^ p2)) + _dot(w2[rs], _ld(p2))
            else:
                ot = _dot(w2[rs], _ld(pc))
            if v1:
                ot = ot + _dot(w1[rs], _ld(pbuf[sb, T // 2:T, hh * 128:(hh + 1) * 128]))
            outs += [ot[8 * j:8 * j + 8] * ls[hh] for j in range(4)]
        o = jnp.concatenate(outs, axis=0).T
        ob_.at[i].bitcast(bf16)[:, _lanes(g)] = o.astype(bf16)

    def step(g, i, gn, inx, r, has_prev, v0, v1, tiles):
        rn = (r + 1) % 4
        ms = scores_b(r, v0, v1)
        proj_bqk(gn, inx, rn)
        attn_a(g, i, r, has_prev)
        ls = softmax_b(r, ms, v1)
        pv_b(ls, g, i, r, v0, v1)
        proj_aq(gn, inx, rn)
        proj_ak(gn, inx, rn)
        proj_av(gn, inx, rn)
        proj_bv(gn, inx, rn)
        for t in tiles:
            transpose_tile(*t)

    cp_xa(0).wait()
    for p, proj in ((0, proj_aq), (1, proj_ak), (2, proj_av)):
        cp_w(0, p).wait()
        transpose_part(0, p)
        proj(0, 0, 0)
    cp_xb(0).wait()
    cp_w(0, 4).wait()
    cp_w(0, 5).wait()
    proj_bqk(0, 0, 0)
    cp_w(0, 3).wait()
    transpose_part(0, 3)
    proj_bv(0, 0, 0)

    for i in range(4):
        for t in {0: (1,), 1: (2,), 2: (3, 4)}.get(i, ()):
            cp_xa(t).wait()
            cp_xb(t).wait()
        if i == 3:
            cp_w(1, 0).wait()
        step(0, i, 0, i + 1, i, i > 0, i >= 2, i >= 1,
             [(1, 0, c) for c in range(8)] if i == 3 else [])

    def body0(a, carry):
        for u in range(3):
            cp_xa(4 * a + u + 1).wait()
            cp_xb(4 * a + u + 1).wait()

        @pl.when(a < 3)
        def _():
            cp_xa(jnp.minimum(4 * a + 4, NT - 1)).wait()
            cp_xb(jnp.minimum(4 * a + 4, NT - 1)).wait()

        for j in range(1, 4):
            @pl.when(a == j)
            def _():
                for p in ((j,) if j < 3 else (3, 4, 5)):
                    cp_w(1, p).wait()

        for u in range(4):
            i = 4 * a + u
            gn, inx = (0, i + 1) if u < 3 else (a // 3, jnp.where(a == 3, 0, i + 1))
            tiles = [(1, a, c) for c in range(8)][3 * u:3 * u + 3] if u < 3 else []
            step(0, i, gn, inx, u, True, True, True, tiles)
        return carry

    lax.fori_loop(1, 4, body0, 0)

    tsched = {i: [] for i in range(NT)}
    for n in range(32):
        tsched[n * 15 // 32].append(divmod(n, 8))

    def body(g, carry):
        gt = jnp.minimum(g + 1, NG - 1)

        @pl.when(g == 2)
        def _():
            for p in range(6):
                cp_w(3, p).wait()

        for i in range(NT):
            gn, inx = (g, i + 1) if i < NT - 1 else (gt, 0)
            step(g, i, gn, inx, i % 4, i > 0, i >= 2, i >= 1,
                 [(gt, p, c) for p, c in tsched[i]])
        return carry

    for p in range(6):
        cp_w(2, p).wait()
    lax.fori_loop(1, NG, body, 0)

    cp_wo(0).wait()
    cp_wo(1).wait()

    def cp_out(s, slot):
        return pltpu.make_async_copy(ostage.at[slot], out_hbm.at[pl.ds(s * (OT * T), OT * T), :],
                                     sem_out.at[slot])

    def obody(s, carry):
        slot = s % 2

        @pl.when(s >= 2)
        def _():
            cp_out(jnp.maximum(s - 2, 0), slot).wait()

        a_ = _ld(oa_[pl.ds(s * OT, OT)].reshape(OT * T // 2, D))
        b_ = _ld(ob_[pl.ds(s * OT, OT)].reshape(OT * T // 2, D))
        ostage_.at[slot].bitcast(bf16)[:, 0:D] = _dot(a_, _ld(woa_[...])).astype(bf16)
        ostage_.at[slot].bitcast(bf16)[:, D:2 * D] = _dot(b_, _ld(wob_[...])).astype(bf16)
        cp_out(s, slot).start()
        return carry

    nsteps = NT // OT
    lax.fori_loop(0, nsteps - 1, obody, 0)
    sl = nsteps - 1
    slot = sl % 2
    cp_out(sl - 2, slot).wait()
    r0 = sl * OT * T
    tails = []

    def send(rows, cols, n):
        c = pltpu.make_async_copy(ostage.at[slot, pl.ds(rows[0], rows[1]), pl.ds(cols, D)],
                                  out_hbm.at[pl.ds(r0 + rows[0], rows[1]), pl.ds(cols, D)],
                                  sem_tail.at[n])
        c.start()
        tails.append(c)

    ost = ostage_.at[slot].bitcast(bf16)
    ost[:, 0:D] = _dot(_ld(oa_[pl.ds(sl * OT, OT)].reshape(OT * T // 2, D)), _ld(woa_[...])).astype(bf16)
    send((0, OT * T), 0, 0)
    for j in range(OT):
        ost[j * T:(j + 1) * T, D:2 * D] = _dot(_ld(ob_[sl * OT + j]), _ld(wob_[...])).astype(bf16)
        send((j * T, T), D, 1 + j)
    cp_out(sl - 1, (sl - 1) % 2).wait()
    for c in tails:
        c.wait()


@jax.jit
def pallas_concat_heads__sliding_local_dilated__sliding_block__prompt_kernel(
    A_x: jax.Array,
    A_wqkv: jax.Array,
    A_wo: jax.Array,
    B_x: jax.Array,
    B_wqkv: jax.Array,
    B_wo: jax.Array,
):
    B = A_x.shape[0]
    assert A_x.shape == B_x.shape == (1, S, D)
    any_spec = pl.BlockSpec(memory_space=pl.ANY)
    vm = pltpu.VMEM
    scratch = [
        vm((NT, T // 2, D), u32), vm((NT, T // 2, D), u32),
        vm((4, D // 2, D), u32),
        vm((NG, 4, 64, D), u32),
        vm((2, D // 2, D), u32),
        vm((D // 2, D), u32), vm((D // 2, D), u32),
        vm((RA, 128, T), f32), vm((64, RA * 128), u32), vm((64, RA * 128), u32),
        vm((64, 512), u32), vm((64, 512), u32), vm((64, 512), u32),
        vm((2, HPG, 2 * T, T), f32), vm((2, T, HPG * T), u32),
        vm((64, 128), u32),
        vm((NT, T // 2, D), u32), vm((NT, T // 2, D), u32),
        vm((2, OT * T // 2, 2 * D), u32),
        pltpu.SemaphoreType.DMA((NT,)), pltpu.SemaphoreType.DMA((NT,)),
        pltpu.SemaphoreType.DMA((4, 6)),
        pltpu.SemaphoreType.DMA((2,)), pltpu.SemaphoreType.DMA((2,)),
        pltpu.SemaphoreType.DMA((1 + OT,)),
    ]
    out = pl.pallas_call(
        _kernel,
        out_shape=jax.ShapeDtypeStruct((S, 2 * D), bf16),
        in_specs=[any_spec] * 6,
        out_specs=any_spec,
        scratch_shapes=scratch,
        compiler_params=pltpu.CompilerParams(
            vmem_limit_bytes=100 * 1024 * 1024,
            flags={"XLA_TPU_FORCE_LP_LLO_SCHEDULER": True},
            disable_bounds_checks=True,
            disable_semaphore_checks=True,
        ),
        name="concat_heads_kernel",
    )(A_x.reshape(S, D), A_wqkv, A_wo, B_x.reshape(S, D), B_wqkv, B_wo)
    return out.reshape(B, S, 2 * D)
```
